```python
import jax
import jax.numpy as jnp

def _softmax(x, axis=-1):
    return jax.nn.softmax(x, axis=axis)

def _gelu(x):
    return jax.nn.gelu(x, approximate=True)

def _silu(x):
    return jax.nn.silu(x)

def _sigmoid(x):
    return jax.nn.sigmoid(x)

def _layernorm(x, axis=-1, eps=1e-05):
    m = jnp.mean(x, axis=axis, keepdims=True)
    v = jnp.var(x, axis=axis, keepdims=True)
    return (x - m) / jnp.sqrt(v + eps)

def _scatter_add(tgt, idx, src, axis=0):
    return tgt.at[idx].add(src)

def _segment_sum(src, seg, n):
    return jax.ops.segment_sum(src, seg, n)

class _Rng:

    def __init__(self, key):
        self._k = key

    def _next(self):
        self._k, sub = jax.random.split(self._k)
        return sub

    def normal(self, shape):
        return jax.random.normal(self._next(), shape, dtype=jnp.bfloat16)

    def randint(self, lo, hi, shape):
        return jax.random.randint(self._next(), shape, lo, hi, dtype=jnp.int32)

    def uniform(self, shape, lo=0.0, hi=1.0):
        return jax.random.uniform(self._next(), shape, jnp.bfloat16, lo, hi)

    def permutation(self, n):
        return jax.random.permutation(self._next(), n)
kernel_name = 'interleave_layers__linear_kernel_hedgehog__mixer_gmlp__prompt'

def _fwd_setup_inputs():
    _rng = _Rng(jax.random.key(int.from_bytes(__import__("os").urandom(4), "little")))
    _w = lambda a: (lambda t: t.astype(jnp.bfloat16) if jnp.issubdtype(t.dtype, jnp.floating) else t)(jnp.asarray(a))

    def _A_setup():
        B, S, D, H = (1, 2048, 640, 32)
        Dh = D // H
        return {'x': _w((lambda *s: _rng.normal(s) * 0.05)(B, S, D)), 'wqkv': _w((lambda *s: _rng.normal(s) * 0.05)(D, 3 * D)), 'w_phi': _w((lambda *s: _rng.normal(s) * 0.05)(H, Dh, Dh) * Dh ** (-0.5)), 'wo': _w((lambda *s: _rng.normal(s) * 0.05)(D, D))}
    _A_in = _A_setup()

    def _B_setup():
        B, S, D, F = (1, 2048, 640, 1536)
        Fh = F // 2
        return {'x': _w((lambda *s: _rng.normal(s) * 0.05)(B, S, D)), 'w_in': _w((lambda *s: _rng.normal(s) * 0.05)(D, 2 * Fh)), 'w_sp': _w(0.01 * (lambda *s: _rng.normal(s) * 0.05)(S, S)), 'b_sp': _w(1.0 + 0.01 * (lambda *s: _rng.normal(s) * 0.05)(S)), 'w_out': _w((lambda *s: _rng.normal(s) * 0.05)(Fh, D))}
    _B_in = _B_setup()
    return {'A_x': _A_in['x'], 'A_wqkv': _A_in['wqkv'], 'A_w_phi': _A_in['w_phi'], 'A_wo': _A_in['wo'], 'B_x': _B_in['x'], 'B_w_in': _B_in['w_in'], 'B_w_sp': _B_in['w_sp'], 'B_b_sp': _B_in['b_sp'], 'B_w_out': _B_in['w_out']}

def _fwd_reference(A_x, A_wqkv, A_w_phi, A_wo, B_x, B_w_in, B_w_sp, B_b_sp, B_w_out):

    def _A_ref(x, wqkv, w_phi, wo):
        B, S, D = x.shape
        H = 32
        Dh = D // H
        qkv = (lambda x, *d: x.transpose(*d))((x @ wqkv).reshape(B, S, 3, H, Dh), 2, 0, 3, 1, 4)
        q, k, v = (qkv[0], qkv[1], qkv[2])
        pq = jnp.einsum('bhsd,hdf->bhsf', q, w_phi)
        pk = jnp.einsum('bhsd,hdf->bhsf', k, w_phi)
        phi_q = jnp.concatenate([_softmax(pq, axis=-1), _softmax(-pq, axis=-1)], axis=-1)
        phi_k = jnp.concatenate([_softmax(pk, axis=-1), _softmax(-pk, axis=-1)], axis=-1)
        kv = jnp.einsum('bhsf,bhsd->bhfd', phi_k, v)
        z = jnp.einsum('bhsf->bhf', phi_k)
        num = jnp.einsum('bhqf,bhfd->bhqd', phi_q, kv)
        den = jnp.einsum('bhqf,bhf->bhq', phi_q, z)[..., None] + 1e-06
        o = num / den
        return (lambda x, *d: x.transpose(*d))(o, 0, 2, 1, 3).reshape(B, S, D) @ wo

    def _B_ref(x, w_in, w_sp, b_sp, w_out):
        B, S, D = x.shape
        F = w_in.shape[-1]
        Fh = F // 2
        z = _gelu(jnp.einsum('bsd,df->bsf', x, w_in))
        z1 = z[..., :Fh].copy()
        z2 = _layernorm(z[..., Fh:], axis=-1)
        g = jnp.einsum('ts,bsf->btf', w_sp, z2) + b_sp[None, :, None]
        return jnp.einsum('bsf,fd->bsd', z1 * g, w_out)
    x = A_x
    x = x + _A_ref(_layernorm(x, axis=-1), A_wqkv, A_w_phi, A_wo)
    x = x + _B_ref(_layernorm(x, axis=-1), B_w_in, B_w_sp, B_b_sp, B_w_out)
    x = x + _A_ref(_layernorm(x, axis=-1), A_wqkv, A_w_phi, A_wo)
    x = x + _B_ref(_layernorm(x, axis=-1), B_w_in, B_w_sp, B_b_sp, B_w_out)
    return x

def setup_inputs():
    _inp = _fwd_setup_inputs()
    _gk = jax.random.fold_in(jax.random.key(int.from_bytes(__import__("os").urandom(4), "little")), 2 ** 31 - 1)
    _shapes = [[1, 2048, 640]]
    _dtypes = ['bfloat16']
    _gks = jax.random.split(_gk, len(_shapes))
    _gs = [jax.random.normal(k, s, dtype=jnp.dtype(d)) * 0.05 for k, s, d in zip(_gks, _shapes, _dtypes)]
    _inp['grad_out'] = _gs[0]
    return _inp

def reference(A_x, A_wqkv, A_w_phi, A_wo, B_w_in, B_w_sp, B_b_sp, B_w_out, B_x, grad_out):
    _const = dict(B_x=B_x)

    def _f(*_d):
        return _fwd_reference(**{'A_x': _d[0], 'A_wqkv': _d[1], 'A_w_phi': _d[2], 'A_wo': _d[3], 'B_w_in': _d[4], 'B_w_sp': _d[5], 'B_b_sp': _d[6], 'B_w_out': _d[7], **_const})
    _out, _vjp = jax.vjp(_f, A_x, A_wqkv, A_w_phi, A_wo, B_w_in, B_w_sp, B_b_sp, B_w_out)
    _grads = _vjp(grad_out)
    _out0 = jnp.asarray(_out)
    return (_out0, *[jnp.asarray(_g) for _g in _grads])
```

```python
import math

import jax
import jax.numpy as jnp
from jax import lax
import jax.experimental.pallas as pl
import jax.experimental.pallas.tpu as pltpu

S = 2048
D = 640
H = 32
DH = 20
F2 = 1536
FH = 768
TM = 512
NT = S // TM
EPS = 1e-5

NG = 8
HG = H // NG
GV = DH * HG
GF = 2 * GV
GA = GV + 16
NV = GV // 8
NW = 4

f32 = jnp.float32
bf16 = jnp.bfloat16

_NN = (((1,), (0,)), ((), ()))
_NT = (((1,), (1,)), ((), ()))
_TN = (((0,), (0,)), ((), ()))

_GC = math.sqrt(2.0 / math.pi)
_GAC = 0.044715


def _mm(a, b, dims=_NN):
    return lax.dot_general(a, b, dims, preferred_element_type=f32)


def _fold(x, op):
    return op(x, pltpu.roll(x, 4, axis=x.ndim - 2))


def _feats_t(p):
    m = p.shape[1]
    p4 = p.reshape(NG, NV, 8, m)
    mx = _fold(jnp.max(p4, axis=1), jnp.maximum)[:, None]
    mn = _fold(jnp.min(p4, axis=1), jnp.minimum)[:, None]
    ep = jnp.exp(p4 - mx)
    en = jnp.exp(mn - p4)
    rp = (1.0 / _fold(jnp.sum(ep, axis=1), jnp.add))[:, None]
    rn = (1.0 / _fold(jnp.sum(en, axis=1), jnp.add))[:, None]
    return ep * rp, en * rn


def _softmax_bwd_t(ph, dph):
    m = ph.shape[1]
    ph4 = ph.reshape(2, NV, 8, m)
    t = ph4 * dph.reshape(2, NV, 8, m)
    r = t - ph4 * _fold(jnp.sum(t, axis=1), jnp.add)[:, None]
    return (r[0] - r[1]).reshape(GV, m)


def _ln(x):
    n = x.shape[1]
    mu = jnp.sum(x, axis=1, keepdims=True) * (1.0 / n)
    xc = x - mu
    var = jnp.sum(xc * xc, axis=1, keepdims=True) * (1.0 / n)
    rstd = lax.rsqrt(var + EPS)
    return xc * rstd, rstd


def _ln_bwd(dy, xhat, rstd):
    n = dy.shape[1]
    m1 = jnp.sum(dy, axis=1, keepdims=True) * (1.0 / n)
    m2 = jnp.sum(dy * xhat, axis=1, keepdims=True) * (1.0 / n)
    return rstd * (dy - m1 - xhat * m2)


def _gelu(u):
    t = jnp.tanh(_GC * (u + _GAC * u * u * u))
    return 0.5 * u * (1.0 + t)


def _gelu_and_grad(u):
    u2 = u * u
    t = jnp.tanh(_GC * (u + _GAC * u * u2))
    h = 0.5 * (1.0 + t)
    g = u * h
    dg = h + 0.5 * u * (1.0 - t * t) * (_GC * (1.0 + 3.0 * _GAC * u2))
    return g, dg


def _head_mats(wphit_ref, w):
    r = lax.broadcasted_iota(jnp.int32, (2 * GV, 256), 0)
    c = lax.broadcasted_iota(jnp.int32, (2 * GV, 256), 1) + 128 * w
    g = (r >= GV).astype(jnp.int32)
    h = (2 * w + g) * HG + (r & 3)
    j = (r - g * GV) >> 2
    mask = (c >= DH * h) & (c < DH * h + DH)
    sub = lax.broadcasted_iota(jnp.int32, (8, 256), 0)
    wv = wphit_ref[:, 128 * w:128 * w + 256].astype(f32)
    rep = jnp.concatenate(
        [jnp.where(sub < 4,
                   jnp.broadcast_to(wv[2 * t:2 * t + 1, :], (8, 256)),
                   jnp.broadcast_to(wv[2 * t + 1:2 * t + 2, :], (8, 256)))
         for t in range(NV)], axis=0)
    rep = jnp.concatenate([rep, rep], axis=0)
    phit = jnp.where(mask, rep, 0.0).astype(bf16)
    permt = jnp.where(c == DH * h + j, 1.0, 0.0).astype(bf16)
    return phit, mask, permt


def _kv_mask(nrows):
    r = lax.broadcasted_iota(jnp.int32, (GA, GF), 0)
    c = lax.broadcasted_iota(jnp.int32, (GA, GF), 1)
    return ((r & 3) == (c & 3)) & (r < nrows)


def _kernel(
    x0_hbm, wqkv_ref, wphit_ref, wo_ref, win_hbm, wsp_hbm, bsp_ref, wout_hbm, gout_hbm,
    out_hbm, dx_hbm, dwqkv_ref, dwphi_ref, dwo_ref, dwin_hbm, dwsp_hbm, dbsp_ref, dwout_hbm,
    sp_a, sp_phiq, sp_phik, sp_v, sp_o, sp_b, sp_u1, sp_u2, sp_g,
    xf, wpt, wop, win_ref, wsp_ref, wspt_ref, wout_ref,
    a_s, phiq_s, phik_s, v_s, o_s, rden_s, kvt_s, stats,
    b_s, u1_s, u2_s, g_s, z2_s, dg_s,
    g_acc, dwo_acc, dwin_acc, dwout_acc, kv_acc, dkvt_s, dbsp_acc,
    t768, t640, dpq_s, gout_s, stage, bcol,
    sem_io, sem_sp, sem_st,
):
    spill_bufs = dict(
        a=(a_s, sp_a, 0), phiq=(phiq_s, sp_phiq, 1), phik=(phik_s, sp_phik, 2),
        v=(v_s, sp_v, 3), o=(o_s, sp_o, 4), b=(b_s, sp_b, 5), u1=(u1_s, sp_u1, 6),
        u2=(u2_s, sp_u2, 7), g=(g_s, sp_g, 8))

    def spill(name):
        v, h, k = spill_bufs[name]
        return pltpu.make_async_copy(v, h, sem_sp.at[k])

    def reload(name):
        v, h, k = spill_bufs[name]
        return pltpu.make_async_copy(h, v, sem_sp.at[k])

    def rows_of(i):
        return pl.ds(pl.multiple_of(i * TM, TM), TM)

    def ones_rows():
        return jnp.ones((16, TM), bf16)

    def loop(body):
        def wrapped(i, _):
            body(i)
            return 0
        lax.fori_loop(0, NT, wrapped, 0)

    cp_x = pltpu.make_async_copy(x0_hbm, t640, sem_io.at[0])
    cp_win = pltpu.make_async_copy(win_hbm, win_ref, sem_io.at[2])
    cp_wsp = pltpu.make_async_copy(wsp_hbm, wsp_ref, sem_io.at[3])
    cp_wout = pltpu.make_async_copy(wout_hbm, wout_ref, sem_io.at[4])
    cp_g = pltpu.make_async_copy(gout_hbm, gout_s, sem_io.at[1])
    cp_x.start()
    cp_win.start()
    cp_wsp.start()
    cp_wout.start()
    cp_g.start()

    for w in range(NW):
        phit, _, permt = _head_mats(wphit_ref, w)
        r0, c0 = 2 * GV * w, 128 * w
        wpt[r0:r0 + 2 * GV, :] = _mm(
            phit, wqkv_ref[:, c0:c0 + 256], _NT).astype(bf16)
        wpt[640 + r0:640 + r0 + 2 * GV, :] = _mm(
            phit, wqkv_ref[:, 640 + c0:640 + c0 + 256], _NT).astype(bf16)
        wpt[1280 + r0:1280 + r0 + 2 * GV, :] = _mm(
            permt, wqkv_ref[:, 1280 + c0:1280 + c0 + 256], _NT).astype(bf16)
        wop[r0:r0 + 2 * GV, :] = _mm(permt, wo_ref[c0:c0 + 256, :]).astype(bf16)

    bcol[...] = jnp.broadcast_to(bsp_ref[...].astype(f32), (8, S)).T[:, 0:1]

    def a1(l, i):
        rows = rows_of(i)
        xh, rstd = _ln(xf[rows, :])
        a = xh.astype(bf16)
        a_s[rows, :] = a
        stats[l, rows, 0:1] = rstd
        pt = _mm(wpt[...], a, _NT)
        qp, qn = _feats_t(pt[0:640, :])
        kp, kn = _feats_t(pt[640:1280, :])
        v = pt[1280:1920, :].astype(bf16)
        v_s[:, rows] = v
        for g in range(NG):
            phiq_s[g * GF:g * GF + GV, rows] = qp[g].reshape(GV, TM).astype(bf16)
            phiq_s[g * GF + GV:(g + 1) * GF, rows] = qn[g].reshape(GV, TM).astype(bf16)
            kb = jnp.concatenate(
                [kp[g].reshape(GV, TM).astype(bf16), kn[g].reshape(GV, TM).astype(bf16)],
                axis=0)
            phik_s[g * GF:(g + 1) * GF, rows] = kb
            va = jnp.concatenate([v[g * GV:(g + 1) * GV, :], ones_rows()], axis=0)
            kv_acc[g] += _mm(va, kb, _NT)

    def a_mid(l):
        for g in range(NG):
            kvt_s[l, g] = jnp.where(_kv_mask(GV + 8), kv_acc[g], 0.0).astype(bf16)

    def a2(l, i):
        rows = rows_of(i)
        os_ = []
        for g in range(NG):
            na = _mm(kvt_s[l, g], phiq_s[g * GF:(g + 1) * GF, rows])
            rd = 1.0 / (na[GV:GV + 8, :] + 1e-6)
            rden_s[l, g * 8:(g + 1) * 8, rows] = rd
            og = na[0:GV, :].reshape(NV, 8, TM) * rd[None]
            os_.append(og.reshape(GV, TM).astype(bf16))
        ot = jnp.concatenate(os_, axis=0)
        o_s[:, rows] = ot
        xf[rows, :] += _mm(ot, wop[...], _TN)

    def b1(l, i):
        rows = rows_of(i)
        xh, rstd = _ln(xf[rows, :])
        b = xh.astype(bf16)
        b_s[rows, :] = b
        stats[l, rows, 1:2] = rstd
        u = _mm(b, win_ref[...]).astype(bf16)
        u1_s[rows, :] = u[:, 0:FH]
        u2_s[rows, :] = u[:, FH:F2]
        zz = _gelu(u.astype(f32))
        t768[rows, :] = zz[:, 0:FH].astype(bf16)
        z2, rstd2 = _ln(zz[:, FH:F2])
        z2_s[l, rows, :] = z2.astype(bf16)
        stats[l, rows, 2:3] = rstd2

    def b2(l, i):
        rows = rows_of(i)
        g = _mm(wsp_ref[rows, :], z2_s[l]) + bcol[rows, :]
        g_s[rows, :] = g.astype(bf16)
        y = (t768[rows, :].astype(f32) * g).astype(bf16)
        xf[rows, :] += _mm(y, wout_ref[...])

    def bb1(l, i):
        rows = rows_of(i)
        dob = xf[rows, :].astype(bf16)
        dy = _mm(dob, wout_ref[...], _NT)
        z1, dgl = _gelu_and_grad(u1_s[rows, :].astype(f32))
        z1 = z1.astype(bf16).astype(f32)
        g = g_s[rows, :].astype(f32)
        y = (z1 * g).astype(bf16)
        dwout_acc[...] += _mm(y, dob, _TN)
        dg = dy * z1
        dg_s[l, rows, :] = dg.astype(bf16)
        dbsp_acc[rows, :] += jnp.sum(dg, axis=1, keepdims=True)
        t768[rows, :] = (dy * g * dgl).astype(bf16)

    def stage_copy(i, slot):
        return pltpu.make_async_copy(
            stage.at[slot], dwsp_hbm.at[rows_of(i), :], sem_st.at[slot])

    def bb2(l, i):
        rows = rows_of(i)
        dz2 = _mm(wspt_ref[rows, :], dg_s[l])
        z2 = z2_s[l, rows, :].astype(f32)
        dzz = _ln_bwd(dz2, z2, stats[l, rows, 2:3])
        _, dgl = _gelu_and_grad(u2_s[rows, :].astype(f32))
        du = jnp.concatenate([t768[rows, :], (dzz * dgl).astype(bf16)], axis=1)
        db = _mm(du, win_ref[...], _NT)
        b = b_s[rows, :]
        dwin_acc[...] += _mm(b, du, _TN)
        xf[rows, :] += _ln_bwd(db, b.astype(f32), stats[l, rows, 1:2])

    def dwsp_tile(i):
        rows = rows_of(i)
        slot = i % 2

        @pl.when(i >= 2)
        def _():
            stage_copy(i - 2, slot).wait()

        dws = (_mm(dg_s[1, rows, :], z2_s[1], _NT)
               + _mm(dg_s[0, rows, :], z2_s[0], _NT))
        stage[slot] = dws.astype(bf16)
        stage_copy(i, slot).start()

    def ab1(l, i):
        rows = rows_of(i)
        dob = xf[rows, :].astype(bf16)
        dot_ = _mm(wop[...], dob, _NT)
        ot = o_s[:, rows]
        dwo_acc[...] += _mm(ot, dob)
        for g in range(NG):
            rd = rden_s[l, g * 8:(g + 1) * 8, rows]
            do3 = dot_[g * GV:(g + 1) * GV, :].reshape(NV, 8, TM)
            o3 = ot[g * GV:(g + 1) * GV, :].astype(f32).reshape(NV, 8, TM)
            dnum = (do3 * rd[None]).reshape(GV, TM).astype(bf16)
            dden = -_fold(jnp.sum(do3 * o3, axis=0), jnp.add) * rd
            dden = jnp.where(
                lax.broadcasted_iota(jnp.int32, (8, TM), 0) < HG, dden, 0.0)
            dden = jnp.concatenate([dden, jnp.zeros((8, TM), f32)], axis=0)
            dna = jnp.concatenate([dnum, dden.astype(bf16)], axis=0)
            dph = _mm(kvt_s[l, g], dna, _TN)
            phq = phiq_s[g * GF:(g + 1) * GF, rows]
            kv_acc[g] += _mm(dna, phq, _NT)
            dpq_s[g * GV:(g + 1) * GV, rows] = _softmax_bwd_t(
                phq.astype(f32), dph).astype(bf16)

    def ab_mid():
        for g in range(NG):
            dkvt_s[g] = jnp.where(_kv_mask(GV + HG), kv_acc[g], 0.0).astype(bf16)

    def ab2(l, i):
        rows = rows_of(i)
        dpk = []
        dv = []
        for g in range(NG):
            va = jnp.concatenate([v_s[g * GV:(g + 1) * GV, rows], ones_rows()], axis=0)
            dphk = _mm(dkvt_s[g], va, _TN)
            phk = phik_s[g * GF:(g + 1) * GF, rows]
            dv.append(_mm(dkvt_s[g, 0:GV, :], phk).astype(bf16))
            dpk.append(_softmax_bwd_t(phk.astype(f32), dphk).astype(bf16))
        dpt = jnp.concatenate([dpq_s[:, rows]] + dpk + dv, axis=0)
        da = _mm(dpt, wpt[...], _TN)
        a = a_s[rows, :]
        g_acc[...] += _mm(dpt, a)
        xf[rows, :] += _ln_bwd(da, a.astype(f32), stats[l, rows, 0:1])

    def zero(ref):
        ref[...] = jnp.zeros_like(ref)

    zero(kv_acc)
    cp_x.wait()

    def l1(i):
        rows = rows_of(i)
        xf[rows, :] = t640[rows, :].astype(f32)
        a1(0, i)

    loop(l1)
    a_mid(0)
    for n in ('a', 'phiq', 'phik', 'v'):
        spill(n).start()
    cp_win.wait()

    def l2(i):
        a2(0, i)
        b1(0, i)

    loop(l2)
    for n in ('o', 'b', 'u1', 'u2'):
        spill(n).start()
    for n in ('a', 'phiq', 'phik', 'v'):
        spill(n).wait()
    zero(kv_acc)
    cp_wsp.wait()
    cp_wout.wait()

    def l3(i):
        rows = rows_of(i)
        wspt_ref[:, rows] = wsp_ref[rows, :].T
        b2(0, i)
        a1(1, i)

    loop(l3)
    a_mid(1)
    spill('g').start()
    for n in ('o', 'b', 'u1', 'u2'):
        spill(n).wait()

    def l4(i):
        a2(1, i)
        b1(1, i)

    loop(l4)
    spill('g').wait()
    cp_g.wait()
    zero(dwout_acc)
    zero(dbsp_acc)

    def l5(i):
        rows = rows_of(i)
        b2(1, i)
        t640[rows, :] = xf[rows, :].astype(bf16)
        xf[rows, :] = gout_s[rows, :].astype(f32)
        bb1(1, i)

    loop(l5)
    cp_out = pltpu.make_async_copy(t640, out_hbm, sem_io.at[0])
    cp_out.start()
    for n in ('g', 'u1'):
        reload(n).start()
    zero(dwin_acc)
    zero(dwo_acc)
    zero(kv_acc)

    def l6(i):
        bb2(1, i)
        ab1(1, i)

    loop(l6)
    ab_mid()
    for n in ('u2', 'b', 'o', 'phiq'):
        reload(n).start()
    for n in ('g', 'u1'):
        reload(n).wait()
    zero(g_acc)

    def l7(i):
        ab2(1, i)
        bb1(0, i)

    loop(l7)
    for n in ('v', 'phik', 'a'):
        reload(n).start()
    for n in ('u2', 'b', 'o', 'phiq'):
        reload(n).wait()
    zero(kv_acc)
    g_s[0:FH, 0:D] = dwout_acc[...].astype(bf16)
    cp_dwout = pltpu.make_async_copy(g_s.at[0:FH, 0:D], dwout_hbm, sem_io.at[4])
    cp_dwout.start()

    def l80(i):
        dwsp_tile(i)

    loop(l80)

    def l8(i):
        bb2(0, i)
        ab1(0, i)

    loop(l8)
    ab_mid()
    for n in ('v', 'phik', 'a'):
        reload(n).wait()
    u1_s[0:D, :] = dwin_acc[:, 0:FH].astype(bf16)
    u2_s[0:D, :] = dwin_acc[:, FH:F2].astype(bf16)
    cp_dwin1 = pltpu.make_async_copy(u1_s.at[0:D, :], dwin_hbm.at[:, 0:FH], sem_io.at[2])
    cp_dwin2 = pltpu.make_async_copy(u2_s.at[0:D, :], dwin_hbm.at[:, FH:F2], sem_io.at[3])
    cp_dwin1.start()
    cp_dwin2.start()

    def l9(i):
        rows = rows_of(i)
        ab2(0, i)
        gout_s[rows, :] = xf[rows, :].astype(bf16)

    loop(l9)
    cp_dx = pltpu.make_async_copy(gout_s, dx_hbm, sem_io.at[1])
    cp_dx.start()

    er = lax.broadcasted_iota(jnp.int32, (2 * GV, 128), 0)
    ec = lax.broadcasted_iota(jnp.int32, (2 * GV, 128), 1)
    sel = jnp.where(((er - (er >= GV).astype(jnp.int32) * GV) >> 2) == ec,
                    1.0, 0.0).astype(bf16)
    parts = [[None] * NW for _ in range(5)]
    for w in range(NW):
        phit, mask_phi, permt = _head_mats(wphit_ref, w)
        r0, c0 = 2 * GV * w, 128 * w
        gq = g_acc[r0:r0 + 2 * GV, :].astype(bf16)
        gk = g_acc[640 + r0:640 + r0 + 2 * GV, :].astype(bf16)
        gv = g_acc[1280 + r0:1280 + r0 + 2 * GV, :].astype(bf16)
        parts[0][w] = _mm(gq, phit, _TN)
        parts[1][w] = _mm(gk, phit, _TN)
        parts[2][w] = _mm(gv, permt, _TN)
        dphit = (_mm(gq, wqkv_ref[:, c0:c0 + 256])
                 + _mm(gk, wqkv_ref[:, 640 + c0:640 + c0 + 256]))
        dphit = jnp.where(mask_phi, dphit, 0.0).astype(bf16)
        parts[3][w] = _mm(dphit, sel, _TN)
        parts[4][w] = _mm(permt, dwo_acc[r0:r0 + 2 * GV, :].astype(bf16), _TN)

    def _colblock(ps, j):
        lo = ps[j - 1][:, 128:256] if j >= 1 else None
        hi = ps[j][:, 0:128] if j < NW else None
        return hi if lo is None else (lo if hi is None else lo + hi)

    def _rowblock(ps, j):
        lo = ps[j - 1][128:256, :] if j >= 1 else None
        hi = ps[j][0:128, :] if j < NW else None
        return hi if lo is None else (lo if hi is None else lo + hi)

    for j in range(NW + 1):
        for t in range(3):
            dwqkv_ref[:, 640 * t + 128 * j:640 * t + 128 * (j + 1)] = _colblock(
                parts[t], j).astype(bf16)
        dwphi_ref[128 * j:128 * (j + 1), :] = _rowblock(parts[3], j)[:, 0:DH].astype(bf16)
        dwo_ref[128 * j:128 * (j + 1), :] = _rowblock(parts[4], j).astype(bf16)
    dbsp_ref[...] = jnp.broadcast_to(dbsp_acc[...], (S, 128)).T[0:1, :].astype(bf16)

    stage_copy(NT - 2, (NT - 2) % 2).wait()
    stage_copy(NT - 1, (NT - 1) % 2).wait()
    cp_out.wait()
    cp_dwout.wait()
    cp_dwin1.wait()
    cp_dwin2.wait()
    cp_dx.wait()


@jax.jit
def pallas_interleave_layers__linear_kernel_hedgehog__mixer_gmlp__prompt_kernel(
    A_x: jax.Array,
    A_wqkv: jax.Array,
    A_w_phi: jax.Array,
    A_wo: jax.Array,
    B_x: jax.Array,
    B_w_in: jax.Array,
    B_w_sp: jax.Array,
    B_b_sp: jax.Array,
    B_w_out: jax.Array,
    grad_out: jax.Array,
):
    del B_x
    x0 = A_x.reshape(S, D)
    gout = grad_out.reshape(S, D)
    wphit = A_w_phi.reshape(D, DH).T
    bsp = B_b_sp.reshape(1, S)

    vm = pl.BlockSpec(memory_space=pltpu.VMEM)
    hbm = pl.BlockSpec(memory_space=pl.ANY)
    sds = jax.ShapeDtypeStruct

    out_shape = (
        sds((S, D), bf16),
        sds((S, D), bf16),
        sds((D, 3 * D), bf16),
        sds((D, DH), bf16),
        sds((D, D), bf16),
        sds((D, F2), bf16),
        sds((S, S), bf16),
        sds((1, S), bf16),
        sds((FH, D), bf16),
        sds((S, D), bf16), sds((2 * D, S), bf16), sds((2 * D, S), bf16),
        sds((D, S), bf16), sds((D, S), bf16),
        sds((S, D), bf16), sds((S, FH), bf16), sds((S, FH), bf16), sds((S, FH), bf16),
    )
    out_specs = (hbm, hbm, vm, vm, vm, hbm, hbm, vm, hbm) + (hbm,) * 9

    scratch = [
        pltpu.VMEM((S, D), f32),
        pltpu.VMEM((3 * D, D), bf16),
        pltpu.VMEM((D, D), bf16),
        pltpu.VMEM((D, F2), bf16),
        pltpu.VMEM((S, S), bf16),
        pltpu.VMEM((S, S), bf16),
        pltpu.VMEM((FH, D), bf16),
        pltpu.VMEM((S, D), bf16),
        pltpu.VMEM((2 * D, S), bf16),
        pltpu.VMEM((2 * D, S), bf16),
        pltpu.VMEM((D, S), bf16),
        pltpu.VMEM((D, S), bf16),
        pltpu.VMEM((2, NG * 8, S), f32),
        pltpu.VMEM((2, NG, GA, GF), bf16),
        pltpu.VMEM((2, S, 128), f32),
        pltpu.VMEM((S, D), bf16),
        pltpu.VMEM((S, FH), bf16),
        pltpu.VMEM((S, FH), bf16),
        pltpu.VMEM((S, FH), bf16),
        pltpu.VMEM((2, S, FH), bf16),
        pltpu.VMEM((2, S, FH), bf16),
        pltpu.VMEM((3 * D, D), f32),
        pltpu.VMEM((D, D), f32),
        pltpu.VMEM((D, F2), f32),
        pltpu.VMEM((FH, D), f32),
        pltpu.VMEM((NG, GA, GF), f32),
        pltpu.VMEM((NG, GA, GF), bf16),
        pltpu.VMEM((S, 1), f32),
        pltpu.VMEM((S, FH), bf16),
        pltpu.VMEM((S, D), bf16),
        pltpu.VMEM((D, S), bf16),
        pltpu.VMEM((S, D), bf16),
        pltpu.VMEM((2, TM, S), bf16),
        pltpu.VMEM((S, 1), f32),
        pltpu.SemaphoreType.DMA((5,)),
        pltpu.SemaphoreType.DMA((9,)),
        pltpu.SemaphoreType.DMA((2,)),
    ]

    res = pl.pallas_call(
        _kernel,
        out_shape=out_shape,
        in_specs=[hbm, vm, vm, vm, hbm, hbm, vm, hbm, hbm],
        out_specs=out_specs,
        scratch_shapes=scratch,
        compiler_params=pltpu.CompilerParams(vmem_limit_bytes=127 * 1024 * 1024),
    )(x0, A_wqkv, wphit, A_wo, B_w_in, B_w_sp, bsp, B_w_out, gout)

    out, dx, dwqkv, dwphi, dwo, dwin, dwsp, dbsp, dwout = res[:9]
    return (
        out.reshape(1, S, D),
        dx.reshape(1, S, D),
        dwqkv,
        dwphi.reshape(H, DH, DH),
        dwo,
        dwin,
        dwsp,
        dbsp.reshape(S),
        dwout,
    )
```
